```python
import os as _os
_os.environ.setdefault("JAX_PLATFORMS", "cpu")
import jax
import jax.numpy as jnp

def _softmax(x, axis=-1):
    return jax.nn.softmax(x, axis=axis)
def _gelu(x):
    return jax.nn.gelu(x, approximate=True)
def _silu(x):
    return jax.nn.silu(x)
def _sigmoid(x):
    return jax.nn.sigmoid(x)
def _layernorm(x, axis=-1, eps=1e-5):
    m = jnp.mean(x, axis=axis, keepdims=True)
    v = jnp.var(x, axis=axis, keepdims=True)
    return (x - m) / jnp.sqrt(v + eps)
def _scatter_add(tgt, idx, src, axis=0):
    return tgt.at[idx].add(src)
def _segment_sum(src, seg, n):
    return jax.ops.segment_sum(src, seg, n)
class _Rng:
    def __init__(self, key):
        self._k = key
    def _next(self):
        self._k, sub = jax.random.split(self._k)
        return sub
    def normal(self, shape):
        return jax.random.normal(self._next(), shape, dtype=jnp.bfloat16)
    def randint(self, lo, hi, shape):
        return jax.random.randint(self._next(), shape, lo, hi, dtype=jnp.int32)
    def uniform(self, shape, lo=0.0, hi=1.0):
        return jax.random.uniform(self._next(), shape, jnp.bfloat16, lo, hi)
    def permutation(self, n):
        return jax.random.permutation(self._next(), n)


kernel_name = 'concat_heads__sliding_block__grouped_kv_mqa__prompt'

def setup_inputs():
    _rng = _Rng(jax.random.key(int.from_bytes(__import__("os").urandom(4), "little")))
    _w = (lambda a: (lambda t: t.astype(jnp.bfloat16) if jnp.issubdtype(t.dtype, jnp.floating) else t)(jnp.asarray(a)))
    def _A_setup():
        B, S, D = 1, 2048, 576
        return {
            "x": _w((lambda *s: _rng.normal(s) * 0.2)(B, S, D)),
            "wqkv": _w((lambda *s: _rng.normal(s) * 0.2)(D, 3 * D)),
            "wo": _w((lambda *s: _rng.normal(s) * 0.05)(D, D)),
        }
    _A_in = _A_setup()

    def _B_setup():
        B, S, D, H = 1, 2048, 576, 32
        Dh = D // H
        return {
            "x": _w((lambda *s: _rng.normal(s) * 0.05)(B, S, D)),
            "wq": _w((lambda *s: _rng.normal(s) * 1.6)(D, H * Dh)),
            "wk": _w((lambda *s: _rng.normal(s) * 1.6)(D, Dh)),
            "wv": _w((lambda *s: _rng.normal(s) * 0.1)(D, Dh)),
            "wo": _w((lambda *s: _rng.normal(s) * 0.1)(H * Dh, D)),
        }
    _B_in = _B_setup()

    return {
        "A_x": _A_in["x"],
        "A_wqkv": _A_in["wqkv"],
        "A_wo": _A_in["wo"],
        "B_x": _B_in["x"],
        "B_wq": _B_in["wq"],
        "B_wk": _B_in["wk"],
        "B_wv": _B_in["wv"],
        "B_wo": _B_in["wo"],
    }

def reference(A_x, A_wqkv, A_wo, B_x, B_wq, B_wk, B_wv, B_wo):
    def _A_ref(x, wqkv, wo):
        B, S, D = x.shape
        H = 32; Dh = D // H; W = 256
        qkv = (lambda x, *d: x.transpose(*d))((x @ wqkv).reshape(B, S, 3, H, Dh), 2, 0, 3, 1, 4)
        q, k, v = qkv[0], qkv[1], qkv[2]
        scores = jnp.einsum("bhqd,bhkd->bhqk", q, k) * (Dh ** -0.5)
        idx = jnp.arange(S)
        mask = (idx[:, None] - idx[None, :] >= 0) & (idx[:, None] - idx[None, :] < W)
        scores = jnp.where(mask[None, None], scores, -1e9)
        p = _softmax(scores, axis=-1)
        o = jnp.einsum("bhqk,bhkd->bhqd", p, v)
        return (lambda x, *d: x.transpose(*d))(o, 0, 2, 1, 3).reshape(B, S, D) @ wo

    def _B_ref(x, wq, wk, wv, wo):
        B, S, D = x.shape
        H = 32
        Dh = D // H
        q = (lambda x, *d: x.transpose(*d))((x @ wq).reshape(B, S, H, Dh), 0, 2, 1, 3)
        k = x @ wk
        v = x @ wv
        scores = jnp.einsum("bhqd,bkd->bhqk", q, k) * (Dh ** -0.5)
        p = _softmax(scores, axis=-1)
        o = jnp.einsum("bhqk,bkd->bhqd", p, v)
        return (lambda x, *d: x.transpose(*d))(o, 0, 2, 1, 3).reshape(B, S, H * Dh) @ wo

    a = _A_ref(A_x, A_wqkv, A_wo)
    b = _B_ref(B_x, B_wq, B_wk, B_wv, B_wo)
    return jnp.concatenate([a, b], axis=-1)
```

```python
import functools
import numpy as np
import jax
import jax.numpy as jnp
from jax import lax
import jax.experimental.pallas as pl
import jax.experimental.pallas.tpu as pltpu

f32 = jnp.float32
bf16 = jnp.bfloat16
u32 = jnp.uint32

S = 2048
D = 576
H = 32
DH = 18
WIN = 256
NT = S // 128
BQ = 256
NQB = S // BQ
TB = 512
NEG = -1e30

_SCALE = 0.2353515625
_C = float(np.float32(_SCALE * 1.4426950408889634))

NN = (((1,), (0,)), ((), ()))
NT_ = (((1,), (1,)), ((), ()))


def _dot(a, b, dims=NN):
    return lax.dot_general(a, b, dims, preferred_element_type=f32)


def _rb(x):
    return x.astype(bf16).astype(f32)


def _rows(shape):
    return lax.broadcasted_iota(jnp.int32, shape, 0)


def _lanes(shape):
    return lax.broadcasted_iota(jnp.int32, shape, 1)


ONES_ROW = (23, 23, 23, 0)
WIN0 = (0, 16, 32, 48)
OFF = (0, 2, 4, 6)


def kernel(xa_h, wqkv_h, woa_h, xb_h, wqb_h, wkb_h, wvb_h, wob_h, out_h,
           xa, xb, wqkv, woa, wob, wqb, wkb, wvb,
           wqkvt, wqbt, woat, wobt, wkvt,
           qat, vat, qbt, oat, obt, ka, kb_ref, vb_ref,
           sb, sa, ma, bias, stage, sem, xsem, osem):
    cps = {}
    NTB = S // TB

    def x_cp(which, tb):
        src, dst = ((xa_h, xa), (xb_h, xb))[which]
        return pltpu.make_async_copy(src.at[:, pl.ds(pl.multiple_of(tb * TB, TB), TB)], dst.at[tb], xsem.at[which, tb])

    order = [("wqb", wqb_h, wqb), ("wkb", wkb_h, wkb), ("wvb", wvb_h, wvb), ("xb", 1, None),
             ("wqkv", wqkv_h, wqkv), ("xa", 0, None), ("woa", woa_h, woa), ("wob", wob_h, wob)]
    for n, (name, src, dst) in enumerate(order):
        if dst is None:
            for tb in range(NTB):
                x_cp(src, tb).start()
        else:
            cps[name] = pltpu.make_async_copy(src, dst, sem.at[n])
            cps[name].start()

    cps["wqb"].wait()
    wqbt[...] = wqb[...].T
    cps["wkb"].wait()
    cps["wvb"].wait()
    z6 = jnp.zeros((6, D), f32)
    wkvt[...] = jnp.concatenate([wkb[...].astype(f32), z6, wvb[...].astype(f32), z6], axis=0)

    r = _rows((128, 128))
    c = _lanes((128, 128))
    zero = jnp.zeros((128, 128), f32)
    neg = jnp.full((128, 128), NEG, f32)
    bias[0] = neg
    bias[1] = zero
    bias[2] = jnp.where(r > c, 0.0, NEG)
    bias[3] = jnp.where(r <= c, 0.0, NEG)

    def projb(tb, carry):
        x_cp(1, tb).wait()
        x = xb[tb]
        q = _rb(_dot(wqbt[...], x))
        for u in range(TB // BQ):
            qbt[tb * (TB // BQ) + u] = q[:, u * BQ:(u + 1) * BQ]
        kv = _dot(wkvt[...], x)
        kt = _rb(kv[0:24] * _C)
        vt = _rb(kv[24:48])
        row0 = pl.multiple_of(tb * TB, TB)
        rr = _rows((24, TB))
        for j in range(4):
            o = OFF[j]
            if o == 0:
                kj, vj = kt, vt
            else:
                kj = pltpu.roll(kt, o, 0)
                vj = pltpu.roll(vt, o, 0)
            kb_ref[j, pl.ds(row0, TB), :] = kj.T
            vj = jnp.where(rr == ONES_ROW[j], 1.0, vj)
            for u in range(TB // 128):
                vb_ref[j, tb * (TB // 128) + u] = vj[:, u * 128:(u + 1) * 128]
        return carry

    lax.fori_loop(0, S // TB, projb, 0)

    cps["wqkv"].wait()
    wqkvt[...] = wqkv[...].T

    def proja(tb, carry):
        x_cp(0, tb).wait()
        x = xa[tb]
        q = _rb(_dot(wqkvt[0:D, :], x))
        v = _rb(_dot(wqkvt[2 * D:3 * D, :], x))
        for u in range(TB // 128):
            qat[tb * (TB // 128) + u] = q[:, u * 128:(u + 1) * 128]
            vat[tb * (TB // 128) + u] = v[:, u * 128:(u + 1) * 128]
        k = _dot(wqkvt[D:2 * D, :], x) * _C
        k = jnp.concatenate([jnp.zeros((64, TB), f32), k], axis=0).T.astype(bf16)
        row0 = pl.multiple_of(tb * (TB // 2), TB // 2)
        kt = [pltpu.bitcast(k[:, 128 * t:128 * (t + 1)], u32) for t in range(5)]
        ln = _lanes((TB // 2, 128))
        for t in range(5):
            ka[t, pl.ds(row0, TB // 2), :] = kt[t]
        for t in range(4):
            ka[5 + t, pl.ds(row0, TB // 2), :] = jnp.where(ln < 64, kt[t + 1], kt[t])
        return carry

    lax.fori_loop(0, S // TB, proja, 0)

    LA = 4
    NSL = 8

    def a_rhs(i, h):
        g8 = (DH * h) // 8
        o = (DH * h) % 8
        q = qat[i, 8 * g8:8 * g8 + 24, :]
        rr = _rows((24, 128))
        q = jnp.where((rr >= o) & (rr < o + DH), q, 0.0)
        pieces = []
        for vr in range(16):
            k = (vr - (g8 + 8)) % 16
            pieces.append(q[8 * k:8 * k + 8] if k < 3 else jnp.zeros((8, 128), f32))
        return jnp.concatenate(pieces, axis=0).astype(bf16)

    def a_chunk(h):
        t0 = (DH * h + 64) // 128
        t1 = (DH * h + DH - 1 + 64) // 128
        return t0 if t0 == t1 else 5 + t0

    def a_tiles(i):
        case = jnp.minimum(i, 2)
        bu = jnp.where(case == 2, 2, 0)
        bf = jnp.where(case == 0, 0, 1)
        return [(jnp.maximum(i - 2, 0), bu), (jnp.maximum(i - 1, 0), bf), (i, 3)]

    def a_qk(i, h):
        rhs = a_rhs(i, h)
        ch = a_chunk(h)
        slot = h % NSL
        mx = [None, None]
        for n, (kt, bi) in enumerate(a_tiles(i)):
            lhs = pltpu.bitcast(ka[ch, pl.ds(pl.multiple_of(kt * 64, 64), 64), :], bf16)
            s = _dot(lhs, rhs) + bias[bi]
            sa[slot, n] = s
            for v in range(16):
                p = s[8 * v:8 * v + 8]
                mx[v % 2] = p if mx[v % 2] is None else jnp.maximum(mx[v % 2], p)
            yield
        m = jnp.max(jnp.maximum(mx[0], mx[1]), axis=0, keepdims=True)
        ma[slot] = jnp.broadcast_to(m, (8, 128))

    def a_pv(i, h, state):
        slot = h % NSL
        j = h % 4
        g8 = (DH * h) // 8
        m = ma[slot]
        acc = None
        rr = _rows((24, 128))
        for n, (kt, bi) in enumerate(a_tiles(i)):
            s = sa[slot, n]
            p = jnp.exp2(s.reshape(16, 8, 128) - m[None]).reshape(128, 128).astype(bf16)
            v = jnp.where(rr == ONES_ROW[j], 1.0, vat[kt, 8 * g8:8 * g8 + 24, :])
            o = _dot(v, p)
            acc = o if acc is None else acc + o
            yield
        o = acc * (1.0 / acc[ONES_ROW[j]:ONES_ROW[j] + 1, :])
        _write_head(oat, i, 8 * g8, j, o, state, 128)

    def a_body(i, carry):
        state = {}
        for step in range(H):
            gq = a_qk(i, step)
            if step < LA:
                gp = a_pv(jnp.maximum(i - 1, 0), H - LA + step, state)
            else:
                gp = a_pv(i, step - LA, state)
            for _ in range(3):
                next(gq)
                next(gp)
            for g in (gq, gp):
                for _ in g:
                    pass
        return carry

    sa[...] = jnp.zeros(sa.shape, f32)
    ma[...] = jnp.zeros(ma.shape, f32)
    lax.fori_loop(0, NT, a_body, 0)
    st = {}
    for step in range(LA):
        for _ in a_pv(NT - 1, H - LA + step, st):
            pass

    HU = 8
    NSB = 4

    def b_qk(t, j, slot):
        qb = t // H
        g = (t % H) // 4
        row0 = pl.multiple_of(72 * g + WIN0[j], 8)
        q = qbt[qb, pl.ds(row0, 24), :]
        mx = [None, None]
        for kb in range(NT):
            s = _dot(kb_ref[j, 128 * kb:128 * (kb + 1), :], q)
            sb[slot, 128 * kb:128 * (kb + 1), :] = s
            for v in range(16):
                p = s[8 * v:8 * v + 8]
                mx[v % 2] = p if mx[v % 2] is None else jnp.maximum(mx[v % 2], p)
            yield
        m = jnp.max(jnp.maximum(mx[0], mx[1]), axis=0, keepdims=True)
        yield jnp.broadcast_to(m, (8, BQ))

    def b_pv(t, j, slot, m, state):
        qb = t // H
        g = (t % H) // 4
        acc = None
        for kb in range(NT):
            s = sb[slot, 128 * kb:128 * (kb + 1), :]
            p = jnp.exp2(s.reshape(16, 8, BQ) - m[None]).reshape(128, BQ).astype(bf16)
            o = _dot(vb_ref[j, kb], p)
            acc = o if acc is None else acc + o
            yield
        o = acc * (1.0 / acc[ONES_ROW[j]:ONES_ROW[j] + 1, :])
        _write_head(obt, qb, pl.multiple_of(72 * g, 8) + WIN0[j], j, o, state, BQ)

    def run(g):
        last = None
        for last in g:
            pass
        return last

    NI = NQB * H
    m0 = run(b_qk(0, 0, 0))
    m1 = run(b_qk(1, 1, 1))

    def b_body(it, carry):
        ms = list(carry)
        state = {}
        for u in range(HU):
            t = it * HU + u
            tq = jnp.minimum(t + 2, NI - 1)
            gq = b_qk(tq, (u + 2) % 4, (u + 2) % NSB)
            gp = b_pv(t, u % 4, u % NSB, ms[0], state)
            for _ in range(NT):
                next(gq)
                next(gp)
            mn = run(gq)
            run(gp)
            ms = [ms[1], mn]
        return tuple(ms)

    lax.fori_loop(0, NI // HU, b_body, (m0, m1))

    cps["woa"].wait()
    cps["wob"].wait()
    woat[...] = woa[...].T
    wobt[...] = wob[...].T

    def out_cp(qb):
        return pltpu.make_async_copy(stage.at[qb % 2], out_h.at[pl.ds(qb * BQ, BQ), :], osem.at[qb % 2])

    for qb in range(NQB):
        oa = jnp.concatenate([oat[2 * qb], oat[2 * qb + 1]], axis=1).astype(bf16)
        ob = obt[qb].astype(bf16)
        ya = _dot(woat[...], oa)
        yb = _dot(wobt[...], ob)
        y = jnp.concatenate([ya, yb], axis=0).T.astype(bf16)
        if qb >= 2:
            out_cp(qb - 2).wait()
        stage[qb % 2] = y
        out_cp(qb).start()
    out_cp(NQB - 2).wait()
    out_cp(NQB - 1).wait()


def _write_head(ref, idx, row0, j, o, state, width):
    first = o[0:8]
    if j > 0:
        first = jnp.where(_rows((8, width)) < OFF[j], state["carry"], first)
    if j < 3:
        ref[idx, pl.ds(row0, 16), :] = jnp.concatenate([first, o[8:16]], axis=0)
        state["carry"] = o[16:24]
    else:
        ref[idx, pl.ds(row0, 24), :] = jnp.concatenate([first, o[8:24]], axis=0)


@jax.jit
def pallas_concat_heads__sliding_block__grouped_kv_mqa__prompt_kernel(
        A_x, A_wqkv, A_wo, B_x, B_wq, B_wk, B_wv, B_wo):
    any_spec = pl.BlockSpec(memory_space=pltpu.HBM)
    V = pltpu.VMEM
    scratch = [
        V((S // TB, D, TB), bf16), V((S // TB, D, TB), bf16), V((D, 3 * D), bf16), V((D, D), bf16), V((D, D), bf16),
        V((D, D), bf16), V((DH, D), bf16), V((DH, D), bf16),
        V((3 * D, D), bf16), V((D, D), bf16), V((D, D), bf16), V((D, D), bf16), V((48, D), f32),
        V((NT, D, 128), f32), V((NT, D, 128), f32), V((NQB, D, BQ), f32),
        V((NT, D, 128), f32), V((NQB, D, BQ), f32),
        V((9, S // 2, 128), u32), V((4, S, 24), f32), V((4, NT, 24, 128), f32),
        V((4, S, BQ), f32), V((8, 3, 128, 128), f32), V((8, 8, 128), f32), V((4, 128, 128), f32),
        V((2, BQ, 2 * D), bf16),
        pltpu.SemaphoreType.DMA((8,)), pltpu.SemaphoreType.DMA((2, S // TB)), pltpu.SemaphoreType.DMA((2,)),
    ]
    out = pl.pallas_call(
        kernel,
        out_shape=jax.ShapeDtypeStruct((S, 2 * D), bf16),
        in_specs=[any_spec] * 8,
        out_specs=any_spec,
        scratch_shapes=scratch,
        name="main",
        compiler_params=pltpu.CompilerParams(vmem_limit_bytes=110 * 1024 * 1024),
    )(A_x[0].T, A_wqkv, A_wo, B_x[0].T, B_wq, B_wk.T, B_wv.T, B_wo)
    return out.reshape(1, S, 2 * D)
```

```python
import numpy as np
import jax
import jax.numpy as jnp
from jax import lax
import jax.experimental.pallas as pl
import jax.experimental.pallas.tpu as pltpu

f32 = jnp.float32
bf16 = jnp.bfloat16
u32 = jnp.uint32

S = 2048
D = 576
H = 32
DH = 18
NT = S // 128
BQ = 256
NQB = S // BQ
TB = 512
NTB = S // TB
NEG = -1e30
HU = 12
TAIL = 4
LA0 = 6
NG = 18
WST = 2
NPRE = 12
LA = 4
UNROLL_PB = 0
UNROLL_PA = 0

_SCALE = 0.2353515625
_C = float(np.float32(_SCALE * 1.4426950408889634))

NN = (((1,), (0,)), ((), ()))


def _dot(a, b):
    return lax.dot_general(a, b, NN, preferred_element_type=f32)


def _rb(x):
    return x.astype(bf16).astype(f32)


def _rows(shape):
    return lax.broadcasted_iota(jnp.int32, shape, 0)


def _lanes(shape):
    return lax.broadcasted_iota(jnp.int32, shape, 1)


ONES_ROW = (23, 23, 23, 0)
WIN0 = (0, 16, 32, 48)
OFF = (0, 2, 4, 6)


def _run(g):
    last = None
    for last in g:
        pass
    return last


def _write_head(ref, idx, row0, j, o, state, width):
    first = o[0:8]
    if j > 0:
        first = jnp.where(_rows((8, width)) < OFF[j], state["carry"], first)
    if j < 3:
        ref[idx, pl.ds(row0, 16), :] = jnp.concatenate([first, o[8:16]], axis=0)
        state["carry"] = o[16:24]
    else:
        ref[idx, pl.ds(row0, 24), :] = jnp.concatenate([first, o[8:24]], axis=0)


def _maxfold(mx, s, n=2):
    for v in range(s.shape[0] // 8):
        p = s[8 * v:8 * v + 8]
        mx[v % n] = p if mx[v % n] is None else jnp.maximum(mx[v % n], p)


def kernel(xa_h, wqkv_h, woa_h, xb_h, wqb_h, wkb_h, wvb_h, wob_h, out_h,
           xa, xb, wqkv, woa, wob, wqb, wkb, wvb,
           wqkvt, wqbt, woat, wobt, wkvt,
           qat, vat, qbt, oat, obt, ka, kb_ref, vb_ref,
           sb, sa, ma, bias, yt, stage, kbc, qbc, sem, xsem, osem):
    def x_cp(which, tb):
        src, dst = ((xa_h, xa), (xb_h, xb))[which]
        return pltpu.make_async_copy(src.at[:, pl.ds(pl.multiple_of(tb * TB, TB), TB)], dst.at[tb], xsem.at[which, tb])

    wcp = {}
    for n, (name, src, dst) in enumerate([("wqb", wqb_h, wqb), ("wkb", wkb_h, wkb), ("wvb", wvb_h, wvb),
                                          ("wqkv", wqkv_h, wqkv), ("woa", woa_h, woa), ("wob", wob_h, wob)]):
        wcp[name] = pltpu.make_async_copy(src, dst, sem.at[n])
    wcp["wkb"].start()
    wcp["wvb"].start()
    wcp["wqb"].start()
    x_cp(1, 0).start()

    r = _rows((128, 128))
    c = _lanes((128, 128))
    bias[0] = jnp.where(r > c, 0.0, NEG)
    bias[1] = jnp.where(r <= c, 0.0, NEG)

    wcp["wkb"].wait()
    wcp["wvb"].wait()
    z6 = jnp.zeros((6, D), f32)
    wkvt[...] = jnp.concatenate([wkb[...].astype(f32), z6, wvb[...].astype(f32), z6], axis=0)
    wcp["wqb"].wait()
    wqbt[...] = wqb[...].T
    def projb(tb, carry):
        x_cp(1, tb).wait()

        @pl.when(tb + 1 < NTB)
        def _():
            x_cp(1, tb + 1).start()

        @pl.when(tb == WST)
        def _():
            wcp["wqkv"].start()

        @pl.when(tb == NTB - 1)
        def _():
            wcp["woa"].start()
            wcp["wob"].start()

        x = xb[tb]
        kv = _dot(wkvt[...], x)
        q = _rb(_dot(wqbt[...], x))
        kt = jnp.concatenate([kv[0:24] * _C, jnp.zeros((104, TB), f32)], axis=0)
        kb_ref[pl.ds(pl.multiple_of(tb * (TB // 2), TB // 2), TB // 2), :] = pltpu.bitcast(kt.T.astype(bf16), u32)
        vt = _rb(kv[24:48])
        rr = _rows((24, TB))
        for j in range(4):
            vj = vt if OFF[j] == 0 else pltpu.roll(vt, OFF[j], 0)
            vj = jnp.where(rr == ONES_ROW[j], 1.0, vj)
            for u in range(TB // 128):
                vb_ref[j, tb * (TB // 128) + u] = vj[:, u * 128:(u + 1) * 128]
        for u in range(TB // BQ):
            qbt[tb * (TB // BQ) + u] = q[:, u * BQ:(u + 1) * BQ]
        return carry

    if UNROLL_PB:
        for tb in range(NTB):
            projb(tb, 0)
    else:
        lax.fori_loop(0, NTB, projb, 0)

    NSB = 4
    NI = NQB * H

    def b_qwin(t, j):
        qb = t // H
        g = (t % H) // 4
        row0 = pl.multiple_of(72 * g + WIN0[j], 8)
        q = qbt[qb, pl.ds(row0, 24), :]
        if OFF[j]:
            q = pltpu.roll(q, 24 - OFF[j], 0)
        return q

    def b_qbcast(q, par):
        for d in range(DH):
            qbc[par, d] = jnp.broadcast_to(q[d:d + 1, :], (8, BQ))
            yield

    NMX = 16 - NG
    NMAX = 3

    VS = 1; VE = 13
    QS = 0; QE = 16
    GEN = 1
    VT = 15
    VMODE = 0
    NACC = 1
    VPOS = 0
    VFOLD = 0

    def vsum(g0, l):
        acc = [None] * NACC
        for d in range(DH):
            pr = kbc[d, 8 * g0:8 * (g0 + 1), :] * qbc[par_[0], d, :, 128 * l:128 * (l + 1)]
            a = d % NACC
            acc[a] = pr if acc[a] is None else acc[a] + pr
        r = acc[0]
        for x in acc[1:]:
            r = r + x
        return r
    par_ = [0]

    def b_vchunks(slot, par, mx):
        if VMODE == 0:
            for g0 in (range(NG) if GEN else range(NMX, 16)):
                par_[0] = par
                sv = jnp.concatenate([vsum(g0, l) for l in range(BQ // 128)], axis=1)
                r0 = 8 * g0 if GEN else 128 * VT + 8 * g0
                sb[slot, r0:r0 + 8, :] = sv
                k = {0: g0 % NMAX, 1: 4, 2: 0, 3: NMAX - 1, 4: (g0 + 1) % NMAX}[VFOLD]
                mx[k] = sv if mx[k] is None else jnp.maximum(mx[k], sv)
                yield
        else:
            for g0 in range(0, 16, 2):
                par_[0] = par
                sv0, sv1 = vsum(g0, 1), vsum(g0 + 1, 1)
                r0 = 128 * VT + 8 * g0
                sb[slot, r0:r0 + 8, 128:256] = sv0
                sb[slot, r0 + 8:r0 + 16, 128:256] = sv1
                vm = jnp.maximum(sv0, sv1)
                mx[2] = vm if mx[2] is None else jnp.maximum(mx[2], vm)
                yield

    def b_qk(t, j, slot, q=None, vpu=False, qn=None, par=0):
        if q is None:
            q = b_qwin(t, j)
        rhs = jnp.concatenate([q, jnp.zeros((104, BQ), f32)], axis=0).astype(bf16)
        mx = [None] * 5
        lo = [None]
        gv = b_vchunks(slot, par, mx) if vpu else iter(())
        gn = b_qbcast(qn, 1 - par) if qn is not None else iter(())
        nchunks = NG if VMODE == 0 else 8
        cnt = [0, 0]

        def adv(kb):
            fr = min(max((kb + 1 - VS) / (VE - VS), 0.0), 1.0)
            qr = min(max((kb + 1 - QS) / (QE - QS), 0.0), 1.0)
            while vpu and cnt[0] < int(fr * nchunks + 1e-6):
                next(gv)
                cnt[0] += 1
            while cnt[1] < int(qr * DH + 1e-6):
                next(gn, None)
                cnt[1] += 1
        for kb in range(NT):
            if VPOS == 1:
                adv(kb)
            if vpu and kb == VT and VMODE == 1:
                s = _dot(pltpu.bitcast(kb_ref[64 * kb:64 * kb + 64, :], bf16), rhs[:, 0:128])
                sb[slot, 128 * kb:128 * kb + 128, 0:128] = s
                t2 = [None, None]
                _maxfold(t2, s)
                lo[0] = jnp.maximum(t2[0], t2[1])
            elif GEN and vpu:
                r0 = max(128 * kb, 8 * NG)
                nr = 128 * (kb + 1) - r0
                if nr > 0:
                    s = _dot(pltpu.bitcast(kb_ref[r0 // 2:(r0 + nr) // 2, :], bf16), rhs)
                    sb[slot, r0:r0 + nr, :] = s
                    _maxfold(mx, s, NMAX)
            else:
                nr = 128 if (kb != VT or not vpu) else 8 * NMX
                if nr:
                    s = _dot(pltpu.bitcast(kb_ref[64 * kb:64 * kb + nr // 2, :], bf16), rhs)
                    sb[slot, 128 * kb:128 * kb + nr, :] = s
                    _maxfold(mx, s, NMAX)
            if VPOS == 0:
                adv(kb)
            yield
        mm = None
        for a in mx:
            if a is not None:
                mm = a if mm is None else jnp.maximum(mm, a)
        m = jnp.max(mm, axis=0, keepdims=True)
        yield jnp.broadcast_to(m, (8, BQ))

    def b_pv(t, j, slot, m, state):
        qb = t // H
        g = (t % H) // 4
        acc = None
        for kb in range(NT):
            s = sb[slot, 128 * kb:128 * (kb + 1), :]
            p = jnp.exp2(s.reshape(16, 8, BQ) - m[None]).reshape(128, BQ).astype(bf16)
            o = _dot(vb_ref[j, kb], p)
            acc = o if acc is None else acc + o
            yield
        o = acc * (1.0 / acc[ONES_ROW[j]:ONES_ROW[j] + 1, :])
        _write_head(obt, qb, pl.multiple_of(72 * g, 8) + WIN0[j], j, o, state, BQ)

    def weight_transposes():
        for name, src, dst in (("wqkv", wqkv, wqkvt), ("woa", woa, woat), ("wob", wob, wobt)):
            wcp[name].wait()
            n = src.shape[1]
            for c0 in range(0, n, 128):
                c1 = min(c0 + 128, n)
                dst[c0:c1, :] = src[:, c0:c1].T
                yield

    filler = weight_transposes()
    ms0 = []
    nf = 0
    for t in range(2):
        gq = b_qk(t, t, t)
        for kb in range(NT):
            next(gq)
            while nf < ((t * NT + kb + 1) * NPRE) // (2 * NT):
                next(filler)
                nf += 1
        ms0.append(_run(gq))
    m0, m1 = ms0
    if NG:
        for tt in range((NG + 15) // 16 if GEN else 1):
            vt_ = tt if GEN else VT
            kl = pltpu.bitcast(kb_ref[64 * vt_:64 * (vt_ + 1), :], bf16).astype(f32)
            for d in range(DH):
                kbc[d, 128 * tt:128 * (tt + 1), :] = jnp.broadcast_to(kl[:, d:d + 1], (128, 128))
        _run(b_qbcast(b_qwin(2, 2), 0))
    for tb in range(NTB):
        x_cp(0, tb).start()

    def b_body(it, carry, last=False):
        ms = list(carry)
        state = {}
        n = TAIL if last else HU
        qcur = None
        for u in range(n):
            t = it * HU + u
            gp = b_pv(t, u % 4, u % NSB, ms[0], state)
            if last and u >= n - 2:
                _run(gp)
                ms = [ms[1], None]
                continue
            if NG:
                qn = b_qwin(jnp.minimum(t + 3, NI - 1), (u + 3) % 4)
                gq = b_qk(t + 2, (u + 2) % 4, (u + 2) % NSB, q=qcur, vpu=True, qn=qn, par=u % 2)
                qcur = qn
            else:
                gq = b_qk(t + 2, (u + 2) % 4, (u + 2) % NSB)
            for kb in range(NT):
                if 0:
                    next(gp)
                    next(gq)
                else:
                    next(gq)
                    next(gp)
                if last and kb % 3 == 1:
                    next(filler, None)
            mn = _run(gq)
            _run(gp)
            ms = [ms[1], mn]
        if last:
            _run(filler)
        return tuple(ms)

    assert (NI - TAIL) % HU == 0
    carry = lax.fori_loop(0, (NI - TAIL) // HU, b_body, (m0, m1))
    b_body((NI - TAIL) // HU, carry, last=True)

    def proja(tb, carry):
        x_cp(0, tb).wait()
        x = xa[tb]
        k = _dot(wqkvt[D:2 * D, :], x) * _C
        q = _rb(_dot(wqkvt[0:D, :], x))
        v = _rb(_dot(wqkvt[2 * D:3 * D, :], x))
        k = jnp.concatenate([jnp.zeros((64, TB), f32), k], axis=0).T.astype(bf16)
        row0 = pl.multiple_of(tb * (TB // 2), TB // 2)
        kt = [pltpu.bitcast(k[:, 128 * t:128 * (t + 1)], u32) for t in range(5)]
        ln = _lanes((TB // 2, 128))
        for t in range(5):
            ka[t, pl.ds(row0, TB // 2), :] = kt[t]
        for t in range(4):
            ka[5 + t, pl.ds(row0, TB // 2), :] = jnp.where(ln < 64, kt[t + 1], kt[t])
        for u in range(TB // 128):
            qat[tb * (TB // 128) + u] = q[:, u * 128:(u + 1) * 128]
            vat[tb * (TB // 128) + u] = v[:, u * 128:(u + 1) * 128]
        return carry

    if UNROLL_PA:
        for tb in range(NTB):
            proja(tb, 0)
    else:
        lax.fori_loop(0, NTB, proja, 0)

    NSL = 8

    def a_rhs(i, h):
        g8 = (DH * h) // 8
        o = (DH * h) % 8
        q = qat[i, 8 * g8:8 * g8 + 24, :]
        rr = _rows((24, 128))
        q = jnp.where((rr >= o) & (rr < o + DH), q, 0.0)
        pieces = []
        for vr in range(16):
            k = (vr - (g8 + 8)) % 16
            pieces.append(q[8 * k:8 * k + 8] if k < 3 else jnp.zeros((8, 128), f32))
        return jnp.concatenate(pieces, axis=0).astype(bf16)

    def a_chunk(h):
        t0 = (DH * h + 64) // 128
        t1 = (DH * h + DH - 1 + 64) // 128
        return t0 if t0 == t1 else 5 + t0

    def a_qk(item, i, h, tiles):
        rhs = a_rhs(i, h)
        ch = a_chunk(h)
        slot = item % NSL
        mx = [None, None]
        for n, (kt, bi) in enumerate(tiles):
            lhs = pltpu.bitcast(ka[ch, pl.ds(pl.multiple_of(kt * 64, 64), 64), :], bf16)
            s = _dot(lhs, rhs)
            if bi is not None:
                s = s + bias[bi]
            sa[slot, n] = s
            _maxfold(mx, s)
            yield
        m = jnp.max(jnp.maximum(mx[0], mx[1]), axis=0, keepdims=True)
        ma[slot] = jnp.broadcast_to(m, (8, 128))

    def a_pv(item, e, h, tiles, state):
        slot = item % NSL
        j = h % 4
        g8 = (DH * h) // 8
        m = ma[slot]
        acc = None
        rr = _rows((24, 128))
        for n, (kt, bi) in enumerate(tiles):
            s = sa[slot, n]
            p = jnp.exp2(s.reshape(16, 8, 128) - m[None]).reshape(128, 128).astype(bf16)
            v = jnp.where(rr == ONES_ROW[j], 1.0, vat[kt, 8 * g8:8 * g8 + 24, :])
            o = _dot(v, p)
            acc = o if acc is None else acc + o
            yield
        o = acc * (1.0 / acc[ONES_ROW[j]:ONES_ROW[j] + 1, :])
        _write_head(oat, e, 8 * g8, j, o, state[e], 128)

    def out_cp(mb, half):
        r0 = half * 128
        return pltpu.make_async_copy(stage.at[mb, r0:r0 + 128, :],
                                     out_h.at[pl.ds(pl.multiple_of(mb * BQ + r0, 128), 128), :], osem.at[mb, half])

    def emit(mb, chunks, send):
        for half in range(2):
            for cidx in chunks:
                stage[mb, 128 * half:128 * (half + 1), 128 * cidx:128 * (cidx + 1)] = \
                    yt[128 * cidx:128 * (cidx + 1), 128 * half:128 * (half + 1)].T.astype(bf16)
                yield
            if send:
                out_cp(mb, half).start()

    NCH = 2 * D // 128
    CH_A = list(range(0, D // 128 + 1))
    CH_B = list(range(D // 128 + 1, NCH))

    def a_body(m, carry, first=False):
        la = LA0 if first else LA

        def tiles(e):
            i = 2 * m + e
            full = [(i - 2, 0), (i - 1, None), (i, 1)]
            if first:
                return [tl for tl in full if tl[0] >= 0]
            return full
        state = [{}, {}]
        items = [(h, e) for h in range(H) for e in range(2)]
        n = len(items)
        go = iter(()) if first else emit(m - 1, CH_A, True)
        ob = obt[m].astype(bf16)
        nd = 4
        ydone = 0
        for step in range(n + la):
            gq = gp = iter(())
            if step < n:
                h, e = items[step]
                gq = a_qk(step, 2 * m + e, h, tiles(e))
            if step >= la:
                h, e = items[step - la]
                gp = a_pv(step - la, e, h, tiles(e), state)
            for _ in range(3):
                next(gq, None)
                next(gp, None)
            _run(gq)
            _run(gp)
            if step < n:
                if step % 4 == 1:
                    next(go, None)
            else:
                while ydone < ((step - n + 1) * nd) // la:
                    ych = D // nd
                    yt[D + ych * ydone:D + ych * (ydone + 1), :] = _dot(wobt[ych * ydone:ych * (ydone + 1), :], ob)
                    ydone += 1
        _run(go)
        oa = jnp.concatenate([oat[0], oat[1]], axis=1).astype(bf16)
        gb = emit(m, CH_B, False)
        for c0 in range(0, D, D // 4):
            yt[c0:c0 + D // 4, :] = _dot(woat[c0:c0 + D // 4, :], oa)
            next(gb, None)
            next(gb, None)
        _run(gb)
        return carry

    a_body(0, 0, first=True)
    lax.fori_loop(1, NQB, a_body, 0)
    _run(emit(NQB - 1, CH_A, True))
    for mb in range(NQB):
        for half in range(2):
            out_cp(mb, half).wait()


@jax.jit
def pallas_concat_heads__sliding_block__grouped_kv_mqa__prompt_kernel(
        A_x, A_wqkv, A_wo, B_x, B_wq, B_wk, B_wv, B_wo):
    any_spec = pl.BlockSpec(memory_space=pltpu.HBM)
    V = pltpu.VMEM
    scratch = [
        V((NTB, D, TB), bf16), V((NTB, D, TB), bf16), V((D, 3 * D), bf16), V((D, D), bf16), V((D, D), bf16),
        V((D, D), bf16), V((DH, D), bf16), V((DH, D), bf16),
        V((3 * D, D), bf16), V((D, D), bf16), V((D, D), bf16), V((D, D), bf16), V((48, D), f32),
        V((NT, D, 128), f32), V((NT, D, 128), f32), V((NQB, D, BQ), f32),
        V((2, D, 128), f32), V((NQB, D, BQ), f32),
        V((9, S // 2, 128), u32), V((S // 2, 128), u32), V((4, NT, 24, 128), f32),
        V((4, S, BQ), f32), V((8, 3, 128, 128), f32), V((8, 8, 128), f32), V((2, 128, 128), f32),
        V((2 * D, BQ), f32), V((NQB, BQ, 2 * D), bf16),
        V((DH, 256, 128), f32), V((2, DH, 8, BQ), f32),
        pltpu.SemaphoreType.DMA((6,)), pltpu.SemaphoreType.DMA((2, NTB)), pltpu.SemaphoreType.DMA((NQB, 2)),
    ]
    out = pl.pallas_call(
        kernel,
        out_shape=jax.ShapeDtypeStruct((S, 2 * D), bf16),
        in_specs=[any_spec] * 8,
        out_specs=any_spec,
        scratch_shapes=scratch,
        name="main",
        compiler_params=pltpu.CompilerParams(vmem_limit_bytes=110 * 1024 * 1024),
    )(A_x[0].T, A_wqkv, A_wo, B_x[0].T, B_wq, B_wk.T, B_wv.T, B_wo)
    return out.reshape(1, S, 2 * D)
```

```python
import numpy as np
import jax
import jax.numpy as jnp
from jax import lax
import jax.experimental.pallas as pl
import jax.experimental.pallas.tpu as pltpu

f32 = jnp.float32
bf16 = jnp.bfloat16
u32 = jnp.uint32

S = 2048
D = 576
H = 32
DH = 18
NT = S // 128
BQ = 256
NQB = S // BQ
TB = 512
NTB = S // TB
NEG = -1e30
HU = 12
TAIL = 4
LA0 = 7
NG = 20
EMB = 4
WST = 2
NPRE = 10
LA = 5
UNROLL_PB = 0
UNROLL_PA = 0

_SCALE = 0.2353515625
_C = float(np.float32(_SCALE * 1.4426950408889634))

NN = (((1,), (0,)), ((), ()))


def _dot(a, b):
    return lax.dot_general(a, b, NN, preferred_element_type=f32)


def _rb(x):
    return x.astype(bf16).astype(f32)


def _rows(shape):
    return lax.broadcasted_iota(jnp.int32, shape, 0)


def _lanes(shape):
    return lax.broadcasted_iota(jnp.int32, shape, 1)


ONES_ROW = (23, 23, 23, 0)
WIN0 = (0, 16, 32, 48)
OFF = (0, 2, 4, 6)


def _run(g):
    last = None
    for last in g:
        pass
    return last


def _write_head(ref, idx, row0, j, o, state, width):
    first = o[0:8]
    if j > 0:
        first = jnp.where(_rows((8, width)) < OFF[j], state["carry"], first)
    if j < 3:
        ref[idx, pl.ds(row0, 16), :] = jnp.concatenate([first, o[8:16]], axis=0)
        state["carry"] = o[16:24]
    else:
        ref[idx, pl.ds(row0, 24), :] = jnp.concatenate([first, o[8:24]], axis=0)


def _maxfold(mx, s, n=2):
    for v in range(s.shape[0] // 8):
        p = s[8 * v:8 * v + 8]
        mx[v % n] = p if mx[v % n] is None else jnp.maximum(mx[v % n], p)


def kernel(xa_h, wqkv_h, woa_h, xb_h, wqb_h, wkb_h, wvb_h, wob_h, out_h,
           xa, xb, wqkv, woa, wob, wqb, wkb, wvb,
           wqkvt, wqbt, woat, wobt, wkvt,
           qat, vat, qbt, oat, obt, ka, kb_ref, vb_ref,
           sb, sa, ma, bias, yt, stage, kbc, qbc, sem, xsem, osem):
    def x_cp(which, tb):
        src, dst = ((xa_h, xa), (xb_h, xb))[which]
        return pltpu.make_async_copy(src.at[:, pl.ds(pl.multiple_of(tb * TB, TB), TB)], dst.at[tb], xsem.at[which, tb])

    wcp = {}
    for n, (name, src, dst) in enumerate([("wqb", wqb_h, wqb), ("wkb", wkb_h, wkb), ("wvb", wvb_h, wvb),
                                          ("wqkv", wqkv_h, wqkv), ("woa", woa_h, woa), ("wob", wob_h, wob)]):
        wcp[name] = pltpu.make_async_copy(src, dst, sem.at[n])
    wcp["wkb"].start()
    wcp["wvb"].start()
    wcp["wqb"].start()
    x_cp(1, 0).start()

    r = _rows((128, 128))
    c = _lanes((128, 128))
    bias[0] = jnp.where(r > c, 0.0, NEG)
    bias[1] = jnp.where(r <= c, 0.0, NEG)

    wcp["wkb"].wait()
    wcp["wvb"].wait()
    z6 = jnp.zeros((6, D), f32)
    wkvt[...] = jnp.concatenate([wkb[...].astype(f32), z6, wvb[...].astype(f32), z6], axis=0)
    wcp["wqb"].wait()
    wqbt[...] = wqb[...].T
    def projb(tb, carry):
        x_cp(1, tb).wait()

        @pl.when(tb + 1 < NTB)
        def _():
            x_cp(1, tb + 1).start()

        @pl.when(tb == WST)
        def _():
            wcp["wqkv"].start()

        @pl.when(tb == NTB - 1)
        def _():
            wcp["woa"].start()
            wcp["wob"].start()

        x = xb[tb]
        kv = _dot(wkvt[...], x)
        q = _rb(_dot(wqbt[...], x))
        kt = jnp.concatenate([kv[0:24] * _C, jnp.zeros((104, TB), f32)], axis=0)
        kb_ref[pl.ds(pl.multiple_of(tb * (TB // 2), TB // 2), TB // 2), :] = pltpu.bitcast(kt.T.astype(bf16), u32)
        vt = _rb(kv[24:48])
        rr = _rows((24, TB))
        for j in range(4):
            vj = vt if OFF[j] == 0 else pltpu.roll(vt, OFF[j], 0)
            vj = jnp.where(rr == ONES_ROW[j], 1.0, vj)
            for u in range(TB // 128):
                vb_ref[j, tb * (TB // 128) + u] = vj[:, u * 128:(u + 1) * 128]
        for u in range(TB // BQ):
            qbt[tb * (TB // BQ) + u] = q[:, u * BQ:(u + 1) * BQ]
        return carry

    if UNROLL_PB:
        for tb in range(NTB):
            projb(tb, 0)
    else:
        lax.fori_loop(0, NTB, projb, 0)

    NSB = 4
    NI = NQB * H

    def b_qwin(t, j):
        qb = t // H
        g = (t % H) // 4
        row0 = pl.multiple_of(72 * g + WIN0[j], 8)
        q = qbt[qb, pl.ds(row0, 24), :]
        if OFF[j]:
            q = pltpu.roll(q, 24 - OFF[j], 0)
        return q

    def b_qbcast(q, par):
        for d in range(DH):
            qbc[par, d] = jnp.broadcast_to(q[d:d + 1, :], (8, BQ))
            yield

    NMX = 16 - NG
    NMAX = 3

    VS = 1; VE = 15
    QS = 4; QE = 16
    GEN = 1
    VT = 15
    VMODE = 0
    NACC = 1
    VPOS = 0
    VFOLD = 0

    def vsum(g0, l):
        acc = [None] * NACC
        for d in range(DH):
            pr = kbc[d, 8 * g0:8 * (g0 + 1), :] * qbc[par_[0], d, :, 128 * l:128 * (l + 1)]
            a = d % NACC
            acc[a] = pr if acc[a] is None else acc[a] + pr
        r = acc[0]
        for x in acc[1:]:
            r = r + x
        return r
    par_ = [0]

    def b_vchunks(slot, par, mx):
        if VMODE == 0:
            for g0 in (range(NG) if GEN else range(NMX, 16)):
                par_[0] = par
                sv = jnp.concatenate([vsum(g0, l) for l in range(BQ // 128)], axis=1)
                r0 = 8 * g0 if GEN else 128 * VT + 8 * g0
                sb[slot, r0:r0 + 8, :] = sv
                k = {0: g0 % NMAX, 1: 4, 2: 0, 3: NMAX - 1, 4: (g0 + 1) % NMAX}[VFOLD]
                mx[k] = sv if mx[k] is None else jnp.maximum(mx[k], sv)
                yield
        else:
            for g0 in range(0, 16, 2):
                par_[0] = par
                sv0, sv1 = vsum(g0, 1), vsum(g0 + 1, 1)
                r0 = 128 * VT + 8 * g0
                sb[slot, r0:r0 + 8, 128:256] = sv0
                sb[slot, r0 + 8:r0 + 16, 128:256] = sv1
                vm = jnp.maximum(sv0, sv1)
                mx[2] = vm if mx[2] is None else jnp.maximum(mx[2], vm)
                yield

    def b_qk(t, j, slot, q=None, vpu=False, qn=None, par=0):
        if q is None:
            q = b_qwin(t, j)
        rhs = jnp.concatenate([q, jnp.zeros((104, BQ), f32)], axis=0).astype(bf16)
        mx = [None] * 5
        lo = [None]
        gv = b_vchunks(slot, par, mx) if vpu else iter(())
        gn = b_qbcast(qn, 1 - par) if qn is not None else iter(())
        nchunks = NG if VMODE == 0 else 8
        cnt = [0, 0]

        def adv(kb):
            fr = min(max((kb + 1 - VS) / (VE - VS), 0.0), 1.0)
            qr = min(max((kb + 1 - QS) / (QE - QS), 0.0), 1.0)
            while vpu and cnt[0] < int(fr * nchunks + 1e-6):
                next(gv)
                cnt[0] += 1
            while cnt[1] < int(qr * DH + 1e-6):
                next(gn, None)
                cnt[1] += 1
        for kb in range(NT):
            if VPOS == 1:
                adv(kb)
            if vpu and kb == VT and VMODE == 1:
                s = _dot(pltpu.bitcast(kb_ref[64 * kb:64 * kb + 64, :], bf16), rhs[:, 0:128])
                sb[slot, 128 * kb:128 * kb + 128, 0:128] = s
                t2 = [None, None]
                _maxfold(t2, s)
                lo[0] = jnp.maximum(t2[0], t2[1])
            elif GEN and vpu:
                r0 = max(128 * kb, 8 * NG)
                nr = 128 * (kb + 1) - r0
                if nr > 0:
                    s = _dot(pltpu.bitcast(kb_ref[r0 // 2:(r0 + nr) // 2, :], bf16), rhs)
                    sb[slot, r0:r0 + nr, :] = s
                    _maxfold(mx, s, NMAX)
            else:
                nr = 128 if (kb != VT or not vpu) else 8 * NMX
                if nr:
                    s = _dot(pltpu.bitcast(kb_ref[64 * kb:64 * kb + nr // 2, :], bf16), rhs)
                    sb[slot, 128 * kb:128 * kb + nr, :] = s
                    _maxfold(mx, s, NMAX)
            if VPOS == 0:
                adv(kb)
            yield
        mm = None
        for a in mx:
            if a is not None:
                mm = a if mm is None else jnp.maximum(mm, a)
        m = jnp.max(mm, axis=0, keepdims=True)
        yield jnp.broadcast_to(m, (8, BQ))

    def b_pv(t, j, slot, m, state):
        qb = t // H
        g = (t % H) // 4
        acc = None
        for kb in range(NT):
            s = sb[slot, 128 * kb:128 * (kb + 1), :]
            p = jnp.exp2(s.reshape(16, 8, BQ) - m[None]).reshape(128, BQ).astype(bf16)
            o = _dot(vb_ref[j, kb], p)
            acc = o if acc is None else acc + o
            yield
        o = acc * (1.0 / acc[ONES_ROW[j]:ONES_ROW[j] + 1, :])
        _write_head(obt, qb, pl.multiple_of(72 * g, 8) + WIN0[j], j, o, state, BQ)

    def weight_transposes():
        for name, src, dst in (("wqkv", wqkv, wqkvt), ("woa", woa, woat), ("wob", wob, wobt)):
            wcp[name].wait()
            n = src.shape[1]
            for c0 in range(0, n, 128):
                c1 = min(c0 + 128, n)
                dst[c0:c1, :] = src[:, c0:c1].T
                yield

    filler = weight_transposes()
    ms0 = []
    nf = 0
    for t in range(2):
        gq = b_qk(t, t, t)
        for kb in range(NT):
            next(gq)
            while nf < ((t * NT + kb + 1) * NPRE) // (2 * NT):
                next(filler)
                nf += 1
        ms0.append(_run(gq))
    m0, m1 = ms0
    if NG:
        for tt in range((NG + 15) // 16 if GEN else 1):
            vt_ = tt if GEN else VT
            kl = pltpu.bitcast(kb_ref[64 * vt_:64 * (vt_ + 1), :], bf16).astype(f32)
            for d in range(DH):
                kbc[d, 128 * tt:128 * (tt + 1), :] = jnp.broadcast_to(kl[:, d:d + 1], (128, 128))
        _run(b_qbcast(b_qwin(2, 2), 0))
    for tb in range(NTB):
        x_cp(0, tb).start()

    def b_body(it, carry, last=False):
        ms = list(carry)
        state = {}
        n = TAIL if last else HU
        qcur = None
        for u in range(n):
            t = it * HU + u
            gp = b_pv(t, u % 4, u % NSB, ms[0], state)
            if last and u >= n - 2:
                _run(gp)
                ms = [ms[1], None]
                continue
            if NG:
                qn = b_qwin(jnp.minimum(t + 3, NI - 1), (u + 3) % 4)
                gq = b_qk(t + 2, (u + 2) % 4, (u + 2) % NSB, q=qcur, vpu=True, qn=qn, par=u % 2)
                qcur = qn
            else:
                gq = b_qk(t + 2, (u + 2) % 4, (u + 2) % NSB)
            for kb in range(NT):
                if 0:
                    next(gp)
                    next(gq)
                else:
                    next(gq)
                    next(gp)
                if last and kb % 3 == 1:
                    next(filler, None)
            mn = _run(gq)
            _run(gp)
            ms = [ms[1], mn]
        if last:
            _run(filler)
        return tuple(ms)

    assert (NI - TAIL) % HU == 0
    carry = lax.fori_loop(0, (NI - TAIL) // HU, b_body, (m0, m1))
    b_body((NI - TAIL) // HU, carry, last=True)

    def proja(tb, carry):
        x_cp(0, tb).wait()
        x = xa[tb]
        k = _dot(wqkvt[D:2 * D, :], x) * _C
        q = _rb(_dot(wqkvt[0:D, :], x))
        v = _rb(_dot(wqkvt[2 * D:3 * D, :], x))
        k = jnp.concatenate([jnp.zeros((64, TB), f32), k], axis=0).T.astype(bf16)
        row0 = pl.multiple_of(tb * (TB // 2), TB // 2)
        kt = [pltpu.bitcast(k[:, 128 * t:128 * (t + 1)], u32) for t in range(5)]
        ln = _lanes((TB // 2, 128))
        for t in range(5):
            ka[t, pl.ds(row0, TB // 2), :] = kt[t]
        for t in range(4):
            ka[5 + t, pl.ds(row0, TB // 2), :] = jnp.where(ln < 64, kt[t + 1], kt[t])
        for u in range(TB // 128):
            qat[tb * (TB // 128) + u] = q[:, u * 128:(u + 1) * 128]
            vat[tb * (TB // 128) + u] = v[:, u * 128:(u + 1) * 128]
        return carry

    if UNROLL_PA:
        for tb in range(NTB):
            proja(tb, 0)
    else:
        lax.fori_loop(0, NTB, proja, 0)

    NSL = 8

    def a_rhs(i, h):
        g8 = (DH * h) // 8
        o = (DH * h) % 8
        q = qat[i, 8 * g8:8 * g8 + 24, :]
        rr = _rows((24, 128))
        q = jnp.where((rr >= o) & (rr < o + DH), q, 0.0)
        pieces = []
        for vr in range(16):
            k = (vr - (g8 + 8)) % 16
            pieces.append(q[8 * k:8 * k + 8] if k < 3 else jnp.zeros((8, 128), f32))
        return jnp.concatenate(pieces, axis=0).astype(bf16)

    def a_chunk(h):
        t0 = (DH * h + 64) // 128
        t1 = (DH * h + DH - 1 + 64) // 128
        return t0 if t0 == t1 else 5 + t0

    def a_qk(item, i, h, tiles):
        rhs = a_rhs(i, h)
        ch = a_chunk(h)
        slot = item % NSL
        mx = [None, None]
        for n, (kt, bi) in enumerate(tiles):
            lhs = pltpu.bitcast(ka[ch, pl.ds(pl.multiple_of(kt * 64, 64), 64), :], bf16)
            s = _dot(lhs, rhs)
            if bi is not None:
                s = s + bias[bi]
            sa[slot, n] = s
            _maxfold(mx, s)
            yield
        m = jnp.max(jnp.maximum(mx[0], mx[1]), axis=0, keepdims=True)
        ma[slot] = jnp.broadcast_to(m, (8, 128))

    def a_pv(item, e, h, tiles, state):
        slot = item % NSL
        j = h % 4
        g8 = (DH * h) // 8
        m = ma[slot]
        acc = None
        rr = _rows((24, 128))
        for n, (kt, bi) in enumerate(tiles):
            s = sa[slot, n]
            p = jnp.exp2(s.reshape(16, 8, 128) - m[None]).reshape(128, 128).astype(bf16)
            v = jnp.where(rr == ONES_ROW[j], 1.0, vat[kt, 8 * g8:8 * g8 + 24, :])
            o = _dot(v, p)
            acc = o if acc is None else acc + o
            yield
        o = acc * (1.0 / acc[ONES_ROW[j]:ONES_ROW[j] + 1, :])
        _write_head(oat, e, 8 * g8, j, o, state[e], 128)

    def out_cp(mb, half):
        r0 = half * 128
        return pltpu.make_async_copy(stage.at[mb, r0:r0 + 128, :],
                                     out_h.at[pl.ds(pl.multiple_of(mb * BQ + r0, 128), 128), :], osem.at[mb, half])

    def emit(mb, chunks, halves, send):
        for half in halves:
            for cidx in chunks:
                stage[mb, 128 * half:128 * (half + 1), 128 * cidx:128 * (cidx + 1)] = \
                    yt[128 * cidx:128 * (cidx + 1), 128 * half:128 * (half + 1)].T.astype(bf16)
                yield
            if half in send:
                out_cp(mb, half).start()

    NCH = 2 * D // 128
    CH_A = list(range(0, D // 128 + 1))
    CH_B = list(range(D // 128 + 1, NCH))

    def a_body(m, carry, first=False):
        la = LA0 if first else LA

        def tiles(e):
            i = 2 * m + e
            full = [(i - 2, 0), (i - 1, None), (i, 1)]
            if first:
                return [tl for tl in full if tl[0] >= 0]
            return full
        state = [{}, {}]
        items = [(h, e) for h in range(H) for e in range(2)]
        n = len(items)
        go = iter(()) if first else emit(m - 1, CH_A, (1,), (1,))
        ob = obt[m].astype(bf16)
        nd = 4
        ydone = 0
        for step in range(n + la):
            gq = gp = iter(())
            if step < n:
                h, e = items[step]
                gq = a_qk(step, 2 * m + e, h, tiles(e))
            if step >= la:
                h, e = items[step - la]
                gp = a_pv(step - la, e, h, tiles(e), state)
            for _ in range(3):
                next(gq, None)
                next(gp, None)
            _run(gq)
            _run(gp)
            if step < n:
                if step % 4 == 1:
                    next(go, None)
            else:
                while ydone < ((step - n + 1) * nd) // la:
                    ych = D // nd
                    yt[D + ych * ydone:D + ych * (ydone + 1), :] = _dot(wobt[ych * ydone:ych * (ydone + 1), :], ob)
                    ydone += 1
        _run(go)
        gb = emit(m, CH_B, (0, 1), ())
        for half in range(2):
            oa = oat[half].astype(bf16)
            for c0 in range(0, D, D // 2):
                yt[c0:c0 + D // 2, 128 * half:128 * (half + 1)] = _dot(woat[c0:c0 + D // 2, :], oa)
                for _ in range(EMB):
                    next(gb, None)
            if half == 0:
                _run(gb)
                gb = emit(m, CH_A, (0,), (0,))
        _run(gb)
        return carry

    a_body(0, 0, first=True)
    lax.fori_loop(1, NQB, a_body, 0)
    _run(emit(NQB - 1, CH_A, (1,), (1,)))
    for mb in range(NQB):
        for half in range(2):
            out_cp(mb, half).wait()


@jax.jit
def pallas_concat_heads__sliding_block__grouped_kv_mqa__prompt_kernel(
        A_x, A_wqkv, A_wo, B_x, B_wq, B_wk, B_wv, B_wo):
    any_spec = pl.BlockSpec(memory_space=pltpu.HBM)
    V = pltpu.VMEM
    scratch = [
        V((NTB, D, TB), bf16), V((NTB, D, TB), bf16), V((D, 3 * D), bf16), V((D, D), bf16), V((D, D), bf16),
        V((D, D), bf16), V((DH, D), bf16), V((DH, D), bf16),
        V((3 * D, D), bf16), V((D, D), bf16), V((D, D), bf16), V((D, D), bf16), V((48, D), f32),
        V((NT, D, 128), f32), V((NT, D, 128), f32), V((NQB, D, BQ), f32),
        V((2, D, 128), f32), V((NQB, D, BQ), f32),
        V((9, S // 2, 128), u32), V((S // 2, 128), u32), V((4, NT, 24, 128), f32),
        V((4, S, BQ), f32), V((8, 3, 128, 128), f32), V((8, 8, 128), f32), V((2, 128, 128), f32),
        V((2 * D, BQ), f32), V((NQB, BQ, 2 * D), bf16),
        V((DH, 256, 128), f32), V((2, DH, 8, BQ), f32),
        pltpu.SemaphoreType.DMA((6,)), pltpu.SemaphoreType.DMA((2, NTB)), pltpu.SemaphoreType.DMA((NQB, 2)),
    ]
    out = pl.pallas_call(
        kernel,
        out_shape=jax.ShapeDtypeStruct((S, 2 * D), bf16),
        in_specs=[any_spec] * 8,
        out_specs=any_spec,
        scratch_shapes=scratch,
        name="main",
        compiler_params=pltpu.CompilerParams(vmem_limit_bytes=110 * 1024 * 1024),
    )(A_x[0].T, A_wqkv, A_wo, B_x[0].T, B_wq, B_wk.T, B_wv.T, B_wo)
    return out.reshape(1, S, 2 * D)
```

```python
import numpy as np
import jax
import jax.numpy as jnp
from jax import lax
import jax.experimental.pallas as pl
import jax.experimental.pallas.tpu as pltpu

f32 = jnp.float32
bf16 = jnp.bfloat16
u32 = jnp.uint32

S = 2048
D = 576
H = 32
DH = 18
NT = S // 128
BQ = 256
NQB = S // BQ
TB = 512
NTB = S // TB
HU = 12
TAIL = 4
NG = 20
NPRE = 10
LA = 5
LA0 = 7
NEG = -1e30

_SCALE = 0.2353515625
_C = float(np.float32(_SCALE * 1.4426950408889634))

NN = (((1,), (0,)), ((), ()))


def _dot(a, b):
    return lax.dot_general(a, b, NN, preferred_element_type=f32)


def _rb(x):
    return x.astype(bf16).astype(f32)


def _rows(shape):
    return lax.broadcasted_iota(jnp.int32, shape, 0)


def _lanes(shape):
    return lax.broadcasted_iota(jnp.int32, shape, 1)


ONES_ROW = (23, 23, 23, 0)
WIN0 = (0, 16, 32, 48)
OFF = (0, 2, 4, 6)


def _run(g):
    last = None
    for last in g:
        pass
    return last


def _write_head(ref, idx, row0, j, o, state, width):
    first = o[0:8]
    if j > 0:
        first = jnp.where(_rows((8, width)) < OFF[j], state["carry"], first)
    if j < 3:
        ref[idx, pl.ds(row0, 16), :] = jnp.concatenate([first, o[8:16]], axis=0)
        state["carry"] = o[16:24]
    else:
        ref[idx, pl.ds(row0, 24), :] = jnp.concatenate([first, o[8:24]], axis=0)


def _maxfold(mx, s, n=2):
    for v in range(s.shape[0] // 8):
        p = s[8 * v:8 * v + 8]
        mx[v % n] = p if mx[v % n] is None else jnp.maximum(mx[v % n], p)


def kernel(xa_h, wqkv_h, woa_h, xb_h, wqb_h, wkb_h, wvb_h, wob_h, out_h,
           xa, xb, wqkv, woa, wob, wqb, wkb, wvb,
           wqkvt, wqbt, woat, wobt, wkvt,
           qat, vat, qbt, oat, obt, ka, kb_ref, vb_ref,
           sb, sa, ma, bias, yt, stage, kbc, qbc, sem, xsem, osem):
    def x_cp(which, tb):
        src, dst = ((xa_h, xa), (xb_h, xb))[which]
        return pltpu.make_async_copy(src.at[:, pl.ds(pl.multiple_of(tb * TB, TB), TB)], dst.at[tb], xsem.at[which, tb])

    wcp = {}
    for n, (name, src, dst) in enumerate([("wqb", wqb_h, wqb), ("wkb", wkb_h, wkb), ("wvb", wvb_h, wvb),
                                          ("wqkv", wqkv_h, wqkv), ("woa", woa_h, woa), ("wob", wob_h, wob)]):
        wcp[name] = pltpu.make_async_copy(src, dst, sem.at[n])
    wcp["wkb"].start()
    wcp["wvb"].start()
    wcp["wqb"].start()
    x_cp(1, 0).start()

    r = _rows((128, 128))
    c = _lanes((128, 128))
    bias[0] = jnp.where(r > c, 0.0, NEG)
    bias[1] = jnp.where(r <= c, 0.0, NEG)

    wcp["wkb"].wait()
    wcp["wvb"].wait()
    z6 = jnp.zeros((6, D), f32)
    wkvt[...] = jnp.concatenate([wkb[...].astype(f32), z6, wvb[...].astype(f32), z6], axis=0)
    wcp["wqb"].wait()
    wqbt[...] = wqb[...].T
    def projb(tb, carry):
        x_cp(1, tb).wait()

        @pl.when(tb + 1 < NTB)
        def _():
            x_cp(1, tb + 1).start()

        @pl.when(tb == 2)
        def _():
            wcp["wqkv"].start()

        @pl.when(tb == NTB - 1)
        def _():
            wcp["woa"].start()
            wcp["wob"].start()

        x = xb[tb]
        kv = _dot(wkvt[...], x)
        q = _rb(_dot(wqbt[...], x))
        kt = jnp.concatenate([kv[0:24] * _C, jnp.zeros((104, TB), f32)], axis=0)
        kb_ref[pl.ds(pl.multiple_of(tb * (TB // 2), TB // 2), TB // 2), :] = pltpu.bitcast(kt.T.astype(bf16), u32)
        vt = _rb(kv[24:48])
        rr = _rows((24, TB))
        for j in range(4):
            vj = vt if OFF[j] == 0 else pltpu.roll(vt, OFF[j], 0)
            vj = jnp.where(rr == ONES_ROW[j], 1.0, vj)
            for u in range(TB // 128):
                vb_ref[j, tb * (TB // 128) + u] = vj[:, u * 128:(u + 1) * 128]
        for u in range(TB // BQ):
            qbt[tb * (TB // BQ) + u] = q[:, u * BQ:(u + 1) * BQ]
        return carry

    lax.fori_loop(0, NTB, projb, 0)

    NSB = 4
    NI = NQB * H

    def b_qwin(t, j):
        qb = t // H
        g = (t % H) // 4
        row0 = pl.multiple_of(72 * g + WIN0[j], 8)
        q = qbt[qb, pl.ds(row0, 24), :]
        if OFF[j]:
            q = pltpu.roll(q, 24 - OFF[j], 0)
        return q

    def b_qbcast(q, par):
        for d in range(DH):
            qbc[par, d] = jnp.broadcast_to(q[d:d + 1, :], (8, BQ))
            yield

    def b_vchunks(slot, par, mx):
        for g0 in range(NG):
            parts = []
            for l in range(BQ // 128):
                acc = None
                for d in range(DH):
                    pr = kbc[d, 8 * g0:8 * (g0 + 1), :] * qbc[par, d, :, 128 * l:128 * (l + 1)]
                    acc = pr if acc is None else acc + pr
                parts.append(acc)
            sv = jnp.concatenate(parts, axis=1)
            sb[slot, 8 * g0:8 * g0 + 8, :] = sv
            k = g0 % 3
            mx[k] = sv if mx[k] is None else jnp.maximum(mx[k], sv)
            yield

    def b_qk(t, j, slot, q=None, qn=None, par=0):
        vpu = qn is not None
        if q is None:
            q = b_qwin(t, j)
        rhs = jnp.concatenate([q, jnp.zeros((104, BQ), f32)], axis=0).astype(bf16)
        mx = [None] * 3
        gv = b_vchunks(slot, par, mx) if vpu else iter(())
        gn = b_qbcast(qn, 1 - par) if vpu else iter(())
        cnt = [0, 0]
        for kb in range(NT):
            r0 = max(128 * kb, 8 * NG) if vpu else 128 * kb
            nr = 128 * (kb + 1) - r0
            if nr > 0:
                s = _dot(pltpu.bitcast(kb_ref[r0 // 2:(r0 + nr) // 2, :], bf16), rhs)
                sb[slot, r0:r0 + nr, :] = s
                _maxfold(mx, s, 3)
            fr = min(max(kb / 14, 0.0), 1.0)
            qr = min(max((kb - 3) / 12, 0.0), 1.0)
            while vpu and cnt[0] < int(fr * NG + 1e-6):
                next(gv)
                cnt[0] += 1
            while cnt[1] < int(qr * DH + 1e-6):
                next(gn, None)
                cnt[1] += 1
            yield
        m = jnp.max(jnp.maximum(jnp.maximum(mx[0], mx[1]), mx[2]), axis=0, keepdims=True)
        yield jnp.broadcast_to(m, (8, BQ))

    def b_pv(t, j, slot, m, state):
        qb = t // H
        g = (t % H) // 4
        acc = None
        for kb in range(NT):
            s = sb[slot, 128 * kb:128 * (kb + 1), :]
            p = jnp.exp2(s.reshape(16, 8, BQ) - m[None]).reshape(128, BQ).astype(bf16)
            o = _dot(vb_ref[j, kb], p)
            acc = o if acc is None else acc + o
            yield
        o = acc * (1.0 / acc[ONES_ROW[j]:ONES_ROW[j] + 1, :])
        _write_head(obt, qb, pl.multiple_of(72 * g, 8) + WIN0[j], j, o, state, BQ)

    def weight_transposes():
        for name, src, dst in (("wqkv", wqkv, wqkvt), ("woa", woa, woat), ("wob", wob, wobt)):
            wcp[name].wait()
            n = src.shape[1]
            for c0 in range(0, n, 128):
                c1 = min(c0 + 128, n)
                dst[c0:c1, :] = src[:, c0:c1].T
                yield

    filler = weight_transposes()
    ms0 = []
    nf = 0
    for t in range(2):
        gq = b_qk(t, t, t)
        for kb in range(NT):
            next(gq)
            while nf < ((t * NT + kb + 1) * NPRE) // (2 * NT):
                next(filler)
                nf += 1
        ms0.append(_run(gq))
    m0, m1 = ms0
    for tt in range((NG + 15) // 16):
        kl = pltpu.bitcast(kb_ref[64 * tt:64 * (tt + 1), :], bf16).astype(f32)
        for d in range(DH):
            kbc[d, 128 * tt:128 * (tt + 1), :] = jnp.broadcast_to(kl[:, d:d + 1], (128, 128))
    _run(b_qbcast(b_qwin(2, 2), 0))
    for tb in range(NTB):
        x_cp(0, tb).start()

    def b_body(it, carry, last=False):
        ms = list(carry)
        state = {}
        n = TAIL if last else HU
        qcur = None
        for u in range(n):
            t = it * HU + u
            gp = b_pv(t, u % 4, u % NSB, ms[0], state)
            if last and u >= n - 2:
                _run(gp)
                ms = [ms[1], None]
                continue
            qn = b_qwin(jnp.minimum(t + 3, NI - 1), (u + 3) % 4)
            gq = b_qk(t + 2, (u + 2) % 4, (u + 2) % NSB, q=qcur, qn=qn, par=u % 2)
            qcur = qn
            for kb in range(NT):
                next(gq)
                next(gp)
                if last and kb % 3 == 1:
                    next(filler, None)
            mn = _run(gq)
            _run(gp)
            ms = [ms[1], mn]
        if last:
            _run(filler)
        return tuple(ms)

    assert (NI - TAIL) % HU == 0
    carry = lax.fori_loop(0, (NI - TAIL) // HU, b_body, (m0, m1))
    b_body((NI - TAIL) // HU, carry, last=True)

    def proja(tb, carry):
        x_cp(0, tb).wait()
        x = xa[tb]
        k = _dot(wqkvt[D:2 * D, :], x) * _C
        q = _rb(_dot(wqkvt[0:D, :], x))
        v = _rb(_dot(wqkvt[2 * D:3 * D, :], x))
        k = jnp.concatenate([jnp.zeros((64, TB), f32), k], axis=0).T.astype(bf16)
        row0 = pl.multiple_of(tb * (TB // 2), TB // 2)
        kt = [pltpu.bitcast(k[:, 128 * t:128 * (t + 1)], u32) for t in range(5)]
        ln = _lanes((TB // 2, 128))
        for t in range(5):
            ka[t, pl.ds(row0, TB // 2), :] = kt[t]
        for t in range(4):
            ka[5 + t, pl.ds(row0, TB // 2), :] = jnp.where(ln < 64, kt[t + 1], kt[t])
        for u in range(TB // 128):
            qat[tb * (TB // 128) + u] = q[:, u * 128:(u + 1) * 128]
            vat[tb * (TB // 128) + u] = v[:, u * 128:(u + 1) * 128]
        return carry

    lax.fori_loop(0, NTB, proja, 0)

    NSL = 8

    def a_rhs(i, h):
        g8 = (DH * h) // 8
        o = (DH * h) % 8
        q = qat[i, 8 * g8:8 * g8 + 24, :]
        rr = _rows((24, 128))
        q = jnp.where((rr >= o) & (rr < o + DH), q, 0.0)
        pieces = []
        for vr in range(16):
            k = (vr - (g8 + 8)) % 16
            pieces.append(q[8 * k:8 * k + 8] if k < 3 else jnp.zeros((8, 128), f32))
        return jnp.concatenate(pieces, axis=0).astype(bf16)

    def a_chunk(h):
        t0 = (DH * h + 64) // 128
        t1 = (DH * h + DH - 1 + 64) // 128
        return t0 if t0 == t1 else 5 + t0

    def a_qk(item, i, h, tiles):
        rhs = a_rhs(i, h)
        ch = a_chunk(h)
        slot = item % NSL
        mx = [None, None]
        for n, (kt, bi) in enumerate(tiles):
            lhs = pltpu.bitcast(ka[ch, pl.ds(pl.multiple_of(kt * 64, 64), 64), :], bf16)
            s = _dot(lhs, rhs)
            if bi is not None:
                s = s + bias[bi]
            sa[slot, n] = s
            _maxfold(mx, s)
            yield
        m = jnp.max(jnp.maximum(mx[0], mx[1]), axis=0, keepdims=True)
        ma[slot] = jnp.broadcast_to(m, (8, 128))

    def a_pv(item, e, h, tiles, state):
        slot = item % NSL
        j = h % 4
        g8 = (DH * h) // 8
        m = ma[slot]
        acc = None
        rr = _rows((24, 128))
        for n, (kt, bi) in enumerate(tiles):
            s = sa[slot, n]
            p = jnp.exp2(s.reshape(16, 8, 128) - m[None]).reshape(128, 128).astype(bf16)
            v = jnp.where(rr == ONES_ROW[j], 1.0, vat[kt, 8 * g8:8 * g8 + 24, :])
            o = _dot(v, p)
            acc = o if acc is None else acc + o
            yield
        o = acc * (1.0 / acc[ONES_ROW[j]:ONES_ROW[j] + 1, :])
        _write_head(oat, e, 8 * g8, j, o, state[e], 128)

    def out_cp(mb, half):
        r0 = half * 128
        return pltpu.make_async_copy(stage.at[mb, r0:r0 + 128, :],
                                     out_h.at[pl.ds(pl.multiple_of(mb * BQ + r0, 128), 128), :], osem.at[mb, half])

    def emit(mb, chunks, halves, send):
        for half in halves:
            for cidx in chunks:
                stage[mb, 128 * half:128 * (half + 1), 128 * cidx:128 * (cidx + 1)] = \
                    yt[128 * cidx:128 * (cidx + 1), 128 * half:128 * (half + 1)].T.astype(bf16)
                yield
            if half in send:
                out_cp(mb, half).start()

    NCH = 2 * D // 128
    CH_A = list(range(0, D // 128 + 1))
    CH_B = list(range(D // 128 + 1, NCH))

    def a_body(m, carry, first=False):
        la = LA0 if first else LA

        def tiles(e):
            i = 2 * m + e
            full = [(i - 2, 0), (i - 1, None), (i, 1)]
            if first:
                return [tl for tl in full if tl[0] >= 0]
            return full
        state = [{}, {}]
        items = [(h, e) for h in range(H) for e in range(2)]
        n = len(items)
        go = iter(()) if first else emit(m - 1, CH_A, (1,), (1,))
        ob = obt[m].astype(bf16)
        nd = 4
        ydone = 0
        for step in range(n + la):
            gq = gp = iter(())
            if step < n:
                h, e = items[step]
                gq = a_qk(step, 2 * m + e, h, tiles(e))
            if step >= la:
                h, e = items[step - la]
                gp = a_pv(step - la, e, h, tiles(e), state)
            for _ in range(3):
                next(gq, None)
                next(gp, None)
            _run(gq)
            _run(gp)
            if step < n:
                if step % 4 == 1:
                    next(go, None)
            else:
                while ydone < ((step - n + 1) * nd) // la:
                    ych = D // nd
                    yt[D + ych * ydone:D + ych * (ydone + 1), :] = _dot(wobt[ych * ydone:ych * (ydone + 1), :], ob)
                    ydone += 1
        _run(go)
        gb = emit(m, CH_B, (0, 1), ())
        for half in range(2):
            oa = oat[half].astype(bf16)
            for c0 in range(0, D, D // 2):
                yt[c0:c0 + D // 2, 128 * half:128 * (half + 1)] = _dot(woat[c0:c0 + D // 2, :], oa)
                for _ in range(4):
                    next(gb, None)
            if half == 0:
                _run(gb)
                gb = emit(m, CH_A, (0,), (0,))
        _run(gb)
        return carry

    a_body(0, 0, first=True)
    lax.fori_loop(1, NQB, a_body, 0)
    _run(emit(NQB - 1, CH_A, (1,), (1,)))
    for mb in range(NQB):
        for half in range(2):
            out_cp(mb, half).wait()


@jax.jit
def pallas_concat_heads__sliding_block__grouped_kv_mqa__prompt_kernel(
        A_x, A_wqkv, A_wo, B_x, B_wq, B_wk, B_wv, B_wo):
    any_spec = pl.BlockSpec(memory_space=pltpu.HBM)
    V = pltpu.VMEM
    scratch = [
        V((NTB, D, TB), bf16), V((NTB, D, TB), bf16), V((D, 3 * D), bf16), V((D, D), bf16), V((D, D), bf16),
        V((D, D), bf16), V((DH, D), bf16), V((DH, D), bf16),
        V((3 * D, D), bf16), V((D, D), bf16), V((D, D), bf16), V((D, D), bf16), V((48, D), f32),
        V((NT, D, 128), f32), V((NT, D, 128), f32), V((NQB, D, BQ), f32),
        V((2, D, 128), f32), V((NQB, D, BQ), f32),
        V((9, S // 2, 128), u32), V((S // 2, 128), u32), V((4, NT, 24, 128), f32),
        V((4, S, BQ), f32), V((8, 3, 128, 128), f32), V((8, 8, 128), f32), V((2, 128, 128), f32),
        V((2 * D, BQ), f32), V((NQB, BQ, 2 * D), bf16),
        V((DH, 256, 128), f32), V((2, DH, 8, BQ), f32),
        pltpu.SemaphoreType.DMA((6,)), pltpu.SemaphoreType.DMA((2, NTB)), pltpu.SemaphoreType.DMA((NQB, 2)),
    ]
    out = pl.pallas_call(
        kernel,
        out_shape=jax.ShapeDtypeStruct((S, 2 * D), bf16),
        in_specs=[any_spec] * 8,
        out_specs=any_spec,
        scratch_shapes=scratch,
        name="main",
        compiler_params=pltpu.CompilerParams(vmem_limit_bytes=110 * 1024 * 1024),
    )(A_x[0].T, A_wqkv, A_wo, B_x[0].T, B_wq, B_wk.T, B_wv.T, B_wo)
    return out.reshape(1, S, 2 * D)
```
